```python
import os as _os
_os.environ.setdefault("JAX_PLATFORMS", "cpu")
import jax
import jax.numpy as jnp

def _softmax(x, axis=-1):
    return jax.nn.softmax(x, axis=axis)
def _gelu(x):
    return jax.nn.gelu(x, approximate=True)
def _silu(x):
    return jax.nn.silu(x)
def _sigmoid(x):
    return jax.nn.sigmoid(x)
def _layernorm(x, axis=-1, eps=1e-5):
    m = jnp.mean(x, axis=axis, keepdims=True)
    v = jnp.var(x, axis=axis, keepdims=True)
    return (x - m) / jnp.sqrt(v + eps)
def _scatter_add(tgt, idx, src, axis=0):
    return tgt.at[idx].add(src)
def _segment_sum(src, seg, n):
    return jax.ops.segment_sum(src, seg, n)
class _Rng:
    def __init__(self, key):
        self._k = key
    def _next(self):
        self._k, sub = jax.random.split(self._k)
        return sub
    def normal(self, shape):
        return jax.random.normal(self._next(), shape, dtype=jnp.bfloat16)
    def randint(self, lo, hi, shape):
        return jax.random.randint(self._next(), shape, lo, hi, dtype=jnp.int32)
    def uniform(self, shape, lo=0.0, hi=1.0):
        return jax.random.uniform(self._next(), shape, jnp.bfloat16, lo, hi)
    def permutation(self, n):
        return jax.random.permutation(self._next(), n)


kernel_name = 'gated_mix__softmax_full_mha__dense_activation_relu__prompt'

def setup_inputs():
    _rng = _Rng(jax.random.key(int.from_bytes(__import__("os").urandom(4), "little")))
    _w = (lambda a: (lambda t: t.astype(jnp.bfloat16) if jnp.issubdtype(t.dtype, jnp.floating) else t)(jnp.asarray(a)))
    def _A_setup():
        B, S, D = 1, 2048, 640
        return {
            "x": _w((lambda *s: _rng.normal(s) * 0.05)(B, S, D)),
            "wqkv": _w((lambda *s: _rng.normal(s) * 0.8)(D, 3 * D)),
            "wo": _w((lambda *s: _rng.normal(s) * 0.05)(D, D)),
        }
    _A_in = _A_setup()

    def _B_setup():
        B, S, D, Dff = 1, 2048, 640, 1536
        return {
            "x": _w((lambda *s: _rng.normal(s) * 0.05)(B, S, D)),
            "w1": _w((lambda *s: _rng.normal(s) * 0.05)(D, Dff)),
            "w2": _w((lambda *s: _rng.normal(s) * 0.05)(Dff, D)),
        }
    _B_in = _B_setup()

    return {
        "A_x": _A_in["x"],
        "A_wqkv": _A_in["wqkv"],
        "A_wo": _A_in["wo"],
        "B_x": _B_in["x"],
        "B_w1": _B_in["w1"],
        "B_w2": _B_in["w2"],
        "gate_w": _w((lambda *s: _rng.normal(s) * 0.05)(640) * 16.0),
    }

def reference(A_x, A_wqkv, A_wo, B_x, B_w1, B_w2, gate_w):
    def _A_ref(x, wqkv, wo):
        B, S, D = x.shape
        H = 32; Dh = D // H
        qkv = (lambda x, *d: x.transpose(*d))((x @ wqkv).reshape(B, S, 3, H, Dh), 2, 0, 3, 1, 4)
        q, k, v = qkv[0], qkv[1], qkv[2]
        scale = Dh ** -0.5
        scores = jnp.einsum("bhqd,bhkd->bhqk", q, k) * scale
        p = _softmax(scores, axis=-1)
        o = jnp.einsum("bhqk,bhkd->bhqd", p, v)
        return (lambda x, *d: x.transpose(*d))(o, 0, 2, 1, 3).reshape(B, S, D) @ wo

    def _B_ref(x, w1, w2):
        h = jnp.einsum("bsd,df->bsf", x, w1)
        zero = jnp.zeros_like(h)
        h = jnp.maximum(h, zero)
        return jnp.einsum("bsf,fd->bsd", h, w2)

    x = A_x
    g = _sigmoid((x * gate_w).sum(-1, keepdims=True))
    a = _A_ref(x, A_wqkv, A_wo)
    b = _B_ref(x, B_w1, B_w2)
    return g * a + (1 - g) * b
```

```python
import functools

import jax
import jax.numpy as jnp
from jax import lax
import jax.experimental.pallas as pl
import jax.experimental.pallas.tpu as pltpu

_H = 32
_LOG2E = 1.4426950408889634
_LANES = 128


def _kernel(x_ref, wqkv_ref, wo_ref, w1_ref, w2_ref, gw_ref, out_ref,
            wk_ref, wqvt_ref, k_ref, qt_ref, vt_ref, ot_ref, s0, s1, z_ref,
            *, S, D, TQ, CK, U):
    H = _H
    DH = D // H
    HPG = _LANES // DH
    NG = -(-H // HPG)
    NQ = S // TQ
    NC = S // CK
    NU = NQ * H
    VR = 24
    f32 = jnp.float32
    bf16 = jnp.bfloat16
    qscale = (DH ** -0.5) * _LOG2E

    def win_start(g):
        if isinstance(g, int):
            return min(g * HPG * DH, D - _LANES)
        return jnp.minimum(g * (HPG * DH), D - _LANES)

    z_ref[0] = 0
    for g in range(NG):
        w0 = D + win_start(g)
        wk_ref[:, g * _LANES:(g + 1) * _LANES] = wqkv_ref[:, w0:w0 + _LANES]
    wqvt_ref[0:D, :] = wqkv_ref[:, 0:D].T
    wqvt_ref[D:2 * D, :] = wqkv_ref[:, 2 * D:3 * D].T
    s1[...] = jnp.zeros_like(s1)
    tail_rows = lax.broadcasted_iota(jnp.int32, (H, 8, S), 1)
    vt_ref[:, 16:24, :] = jnp.where(tail_rows == DH - 16, 1.0, 0.0).astype(f32)

    for r in range(NQ):
        rows = slice(r * TQ, (r + 1) * TQ)
        xr = x_ref[rows, :]
        kk = jnp.dot(xr, wk_ref[...], preferred_element_type=f32)
        for g in range(NG):
            k_ref[g, rows, :] = kk[:, g * _LANES:(g + 1) * _LANES].astype(bf16)
        qv = lax.dot_general(wqvt_ref[...], xr, (((1,), (1,)), ((), ())),
                             preferred_element_type=f32)
        qt_ref[r] = qv[0:D, :] * qscale
        vt = qv[D:2 * D, :].astype(bf16).astype(f32)
        for h in range(H):
            vt_ref[h, 0:DH, rows] = vt[h * DH:(h + 1) * DH, :]

    row_id = lax.broadcasted_iota(jnp.int32, (_LANES, TQ), 0)
    sbuf = (s0, s1)

    def qmask(u):
        h = u % H
        qi = u // H
        g = h // HPG
        w0 = win_start(g)
        off = h * DH - w0
        q = qt_ref[qi, pl.ds(pl.multiple_of(w0, 8), _LANES), :]
        keep = (row_id >= off) & (row_id < off + DH)
        return jnp.where(keep, q, 0.0).astype(bf16), g

    def a_chunk(qm, g, c, s_ref, m):
        s = jnp.dot(k_ref[g, c * CK:(c + 1) * CK, :], qm, preferred_element_type=f32)
        s_ref[0, c * CK:(c + 1) * CK, :] = s
        mc = jnp.max(s.reshape(CK // 8, 8, TQ), axis=0)
        return mc if m is None else jnp.maximum(m, mc)

    def b_chunk(vt, c, s_ref, z, m, acc):
        p = jnp.exp2(s_ref[z, c * CK:(c + 1) * CK, :] - m).astype(bf16)
        o = lax.dot_general(vt[:, c * CK:(c + 1) * CK], p, (((1,), (0,)), ((), ())),
                            preferred_element_type=f32)
        return o if acc is None else acc + o

    def fin(acc, u, odd):
        h = u % H
        qi = u // H
        l = acc[DH:DH + 1, :]
        o = acc[0:DH, :] * (1.0 / l)
        r0 = DH if odd else 0
        ot_ref[qi, h // 2, r0:r0 + DH, :] = o

    def body(j, m_b):
        z = z_ref[0]
        u0 = j * U
        for i in range(U):
            ua = u0 + i
            ub = (u0 + i - 1 + NU) % NU
            qm, g = qmask(ua)
            vt = vt_ref.at[ub % H]
            m_a = None
            acc = None
            for c in range(NC):
                m_a = a_chunk(qm, g, c, sbuf[i % 2], m_a)
                acc = b_chunk(vt, c, sbuf[(i + 1) % 2], z, m_b, acc)
            fin(acc, ub, (i + 1) % 2 == 1)
            m_b = jnp.max(m_a, axis=0, keepdims=True)
        return m_b

    m_b = lax.fori_loop(0, NU // U, body, jnp.zeros((1, TQ), f32))
    z = z_ref[0]
    acc = None
    vt_last = vt_ref.at[H - 1]
    for c in range(NC):
        acc = b_chunk(vt_last, c, s1, z, m_b, acc)
    fin(acc, NU - 1, True)

    gw = gw_ref[...].astype(f32)
    for r in range(NQ):
        rows = slice(r * TQ, (r + 1) * TQ)
        xr = x_ref[rows, :]
        hid = jnp.maximum(jnp.dot(xr, w1_ref[...], preferred_element_type=f32), 0.0)
        b = jnp.dot(hid.astype(bf16), w2_ref[...], preferred_element_type=f32)
        ot = ot_ref[r].reshape(D, TQ).astype(bf16)
        a = lax.dot_general(ot, wo_ref[...], (((0,), (0,)), ((), ())),
                            preferred_element_type=f32)
        gl = jnp.sum(xr.astype(f32) * gw, axis=-1, keepdims=True)
        gate = jax.nn.sigmoid(gl)
        out_ref[rows, :] = (gate * a + (1.0 - gate) * b).astype(out_ref.dtype)


@jax.jit
def pallas_gated_mix__softmax_full_mha__dense_activation_relu__prompt_kernel(
    A_x: jax.Array,
    A_wqkv: jax.Array,
    A_wo: jax.Array,
    B_x: jax.Array,
    B_w1: jax.Array,
    B_w2: jax.Array,
    gate_w: jax.Array,
):
    del B_x
    B, S, D = A_x.shape
    assert B == 1
    H = _H
    DH = D // H
    TQ, CK, U = 512, 128, 4
    NQ = S // TQ
    NG = -(-H // (_LANES // DH))
    f32, bf16 = jnp.float32, jnp.bfloat16

    out = pl.pallas_call(
        functools.partial(_kernel, S=S, D=D, TQ=TQ, CK=CK, U=U),
        out_shape=jax.ShapeDtypeStruct((S, D), A_x.dtype),
        scratch_shapes=[
            pltpu.VMEM((D, NG * _LANES), bf16),
            pltpu.VMEM((2 * D, D), bf16),
            pltpu.VMEM((NG, S, _LANES), bf16),
            pltpu.VMEM((NQ, D, TQ), f32),
            pltpu.VMEM((H, 24, S), f32),
            pltpu.VMEM((NQ, H // 2, 2 * DH, TQ), f32),
            pltpu.VMEM((1, S, TQ), f32),
            pltpu.VMEM((1, S, TQ), f32),
            pltpu.SMEM((1,), jnp.int32),
        ],
        compiler_params=pltpu.CompilerParams(vmem_limit_bytes=100 * 1024 * 1024),
    )(A_x.reshape(S, D), A_wqkv, A_wo, B_w1, B_w2, gate_w.reshape(1, D))
    return out.reshape(B, S, D)
```

```python
import functools

import jax
import jax.numpy as jnp
from jax import lax
import jax.experimental.pallas as pl
import jax.experimental.pallas.tpu as pltpu

_H = 32
_LOG2E = 1.4426950408889634
_LANES = 128


def _kernel(x_hbm, wqkv_hbm, wo_hbm, w1_hbm, w2_hbm, gw_hbm, out_hbm,
            gw_ref, x_ref, wqkv_ref, wo_ref, w1_ref, w2_ref, out_ref,
            wqvt_ref, k_ref, qt_ref, vt_ref, ot_ref, s0, s1, z_ref,
            xsem, wsem, osem,
            *, S, D, TQ, CK, U, TK, TR, SKEW, SC, DEFER, JIT, WQAT, WVAT):
    H = _H
    DH = D // H
    HPG = _LANES // DH
    NG = -(-H // HPG)
    NQ = S // TQ
    NC = S // CK
    NU = NQ * H
    NR = S // TR
    NK = S // TK
    f32 = jnp.float32
    bf16 = jnp.bfloat16
    qscale = (DH ** -0.5) * _LOG2E

    def win_start(g):
        if isinstance(g, int):
            return min(g * HPG * DH, D - _LANES)
        return jnp.minimum(g * (HPG * DH), D - _LANES)

    def rows_of(r, t):
        if isinstance(r, int):
            return pl.ds(r * t, t)
        return pl.ds(pl.multiple_of(r * t, t), t)

    def x_copy(r):
        return pltpu.make_async_copy(x_hbm.at[rows_of(r, TK)], x_ref.at[rows_of(r, TK)], xsem.at[r])

    def wqkv_copy(i):
        cols = pl.ds(i * D, D)
        return pltpu.make_async_copy(wqkv_hbm.at[:, cols], wqkv_ref.at[:, cols], wsem.at[i])

    wo_copy = pltpu.make_async_copy(wo_hbm, wo_ref, wsem.at[3])
    w1_copy = pltpu.make_async_copy(w1_hbm, w1_ref, wsem.at[4])
    w2_copy = pltpu.make_async_copy(w2_hbm, w2_ref, wsem.at[5])
    gw_copy = pltpu.make_async_copy(gw_hbm, gw_ref, wsem.at[6])

    def out_copy(r):
        return pltpu.make_async_copy(out_ref.at[rows_of(r, TR)], out_hbm.at[rows_of(r, TR)], osem.at[r])

    x_copy(0).start()
    wqkv_copy(1).start()
    if JIT:
        for r in range(1, JIT):
            x_copy(r).start()
    else:
        for r in range(1, NK):
            x_copy(r).start()
        wqkv_copy(0).start()
        wqkv_copy(2).start()
    if not DEFER:
        w1_copy.start()
        w2_copy.start()
        wo_copy.start()
        gw_copy.start()

    z_ref[0] = 0
    s1[...] = jnp.zeros_like(s1)
    tail_rows = lax.broadcasted_iota(jnp.int32, (H, 8, S), 1)
    vt_ref[:, 16:24, :] = jnp.where(tail_rows == DH - 16, 1.0, 0.0).astype(f32)

    def kproj(r):
        rows = rows_of(r, TK)
        kk = jnp.dot(x_ref[rows, :], wqkv_ref[:, D:2 * D], preferred_element_type=f32)
        for g in range(NG):
            w0 = win_start(g)
            k_ref[g, rows, :] = kk[:, w0:w0 + _LANES].astype(bf16)

    def qvproj(r):
        rows = rows_of(r, TQ)
        qv = lax.dot_general(wqvt_ref[...], x_ref[rows, :], (((1,), (1,)), ((), ())),
                             preferred_element_type=f32)
        qt_ref[r] = qv[0:D, :] * qscale
        vt = qv[D:2 * D, :].astype(bf16).astype(f32)
        for h in range(H):
            vt_ref[h, 0:DH, rows] = vt[h * DH:(h + 1) * DH, :]

    wqkv_copy(1).wait()

    def k_body(r, c):
        if JIT:
            @pl.when(r + JIT < NK)
            def _():
                x_copy(r + JIT).start()
            @pl.when(r == WQAT)
            def _():
                wqkv_copy(0).start()
            @pl.when(r == WVAT)
            def _():
                wqkv_copy(2).start()
        x_copy(r).wait()
        kproj(r)
        return c
    lax.fori_loop(0, NK - 1, k_body, 0)
    x_copy(NK - 1).wait()
    wqkv_copy(0).wait()
    wqkv_copy(2).wait()
    kproj(NK - 1)
    wqvt_ref[0:D, :] = wqkv_ref[:, 0:D].T
    wqvt_ref[D:2 * D, :] = wqkv_ref[:, 2 * D:3 * D].T

    def qv_body(r, c):
        qvproj(r)
        return c
    lax.fori_loop(0, NQ, qv_body, 0)

    row_id = lax.broadcasted_iota(jnp.int32, (_LANES, TQ), 0)
    sbuf = (s0, s1)

    def qmask(u):
        h = u % H
        qi = u // H
        g = h // HPG
        w0 = win_start(g)
        off = h * DH - w0
        q = qt_ref[qi, pl.ds(pl.multiple_of(w0, 8), _LANES), :]
        keep = (row_id >= off) & (row_id < off + DH)
        return jnp.where(keep, q, 0.0).astype(bf16), g

    def a_chunk(qm, g, c, s_ref, m):
        s = jnp.dot(k_ref[g, c * CK:(c + 1) * CK, :], qm, preferred_element_type=f32)
        s_ref[0, c * CK:(c + 1) * CK, :] = s
        mc = jnp.max(s.reshape(CK // 8, 8, TQ), axis=0)
        return mc if m is None else jnp.maximum(m, mc)

    def b_chunk(vt, c, s_ref, z, m, acc):
        p = jnp.exp2(s_ref[z, c * CK:(c + 1) * CK, :] - m).astype(bf16)
        o = lax.dot_general(vt[:, c * CK:(c + 1) * CK], p, (((1,), (0,)), ((), ())),
                            preferred_element_type=f32)
        return o if acc is None else acc + o

    def fin(acc, u, odd):
        h = u % H
        qi = u // H
        l = acc[DH:DH + 1, :]
        o = acc[0:DH, :] * (1.0 / l)
        r0 = DH if odd else 0
        ot_ref[qi, h // 2, r0:r0 + DH, :] = o

    def body(j, m_b):
        if DEFER:
            @pl.when(j == 1)
            def _():
                w1_copy.start()
                w2_copy.start()
                wo_copy.start()
                gw_copy.start()
        z = z_ref[0]
        u0 = j * U
        for i in range(U):
            ua = u0 + i
            ub = (u0 + i - 1 + NU) % NU
            qm, g = qmask(ua)
            vt = vt_ref.at[ub % H]
            m_a = None
            acc = None
            for c in range(NC + SKEW):
                if c < NC:
                    m_a = a_chunk(qm, g, c, sbuf[i % 2], m_a)
                if c >= SKEW:
                    acc = b_chunk(vt, c - SKEW, sbuf[(i + 1) % 2], z, m_b, acc)
            fin(acc, ub, (i + 1) % 2 == 1)
            m_b = jnp.max(m_a, axis=0, keepdims=True)
        return m_b

    m_b = lax.fori_loop(0, NU // U, body, jnp.zeros((1, TQ), f32))

    w1_copy.wait()
    w2_copy.wait()
    wo_copy.wait()
    gw_copy.wait()
    gw = gw_ref[...].astype(f32).reshape(1, D)
    RPQ = TQ // TR

    def p3(r):
        rows = rows_of(r, TR)
        xr = x_ref[rows, :]
        hid = jnp.maximum(jnp.dot(xr, w1_ref[...], preferred_element_type=f32), 0.0)
        b = jnp.dot(hid.astype(bf16), w2_ref[...], preferred_element_type=f32)
        if RPQ == 1:
            ot = ot_ref[r].reshape(D, TQ).astype(bf16)
        else:
            ot = ot_ref[r // RPQ, :, :, rows_of(r % RPQ, TR)].reshape(D, TR).astype(bf16)
        a = lax.dot_general(ot, wo_ref[...], (((0,), (0,)), ((), ())),
                            preferred_element_type=f32)
        gl = jnp.sum(xr.astype(f32) * gw, axis=-1, keepdims=True)
        gate = jax.nn.sigmoid(gl)
        out_ref[rows, :] = (gate * a + (1.0 - gate) * b).astype(out_ref.dtype)
        out_copy(r).start()

    z = z_ref[0]
    acc = None
    vt_last = vt_ref.at[H - 1]
    for c in range(NC):
        acc = b_chunk(vt_last, c, s1, z, m_b, acc)
    fin(acc, NU - 1, True)
    p3(0)

    def p3_body(r, c):
        p3(r)
        return c
    lax.fori_loop(1, NR, p3_body, 0)
    for r in range(NR):
        out_copy(r).wait()


def make(TQ=512, CK=128, U=4, TK=256, TR=512, SKEW=2, SC=False, DEFER=True, JIT=2, WQAT=1, WVAT=3):
  @jax.jit
  def pallas_gated_mix__softmax_full_mha__dense_activation_relu__prompt_kernel(
    A_x: jax.Array,
    A_wqkv: jax.Array,
    A_wo: jax.Array,
    B_x: jax.Array,
    B_w1: jax.Array,
    B_w2: jax.Array,
    gate_w: jax.Array,
  ):
    del B_x
    B, S, D = A_x.shape
    assert B == 1
    H = _H
    DH = D // H
    DFF = B_w1.shape[1]
    NQ = S // TQ
    NG = -(-H // (_LANES // DH))
    f32, bf16 = jnp.float32, jnp.bfloat16
    anyspec = pl.BlockSpec(memory_space=pl.ANY)

    out = pl.pallas_call(
        functools.partial(_kernel, S=S, D=D, TQ=TQ, CK=CK, U=U, TK=TK, TR=TR, SKEW=SKEW, SC=SC, DEFER=DEFER, JIT=JIT, WQAT=WQAT, WVAT=WVAT),
        out_shape=jax.ShapeDtypeStruct((S, D), A_x.dtype),
        in_specs=[anyspec] * 6,
        out_specs=anyspec,
        scratch_shapes=[
            pltpu.VMEM((D,), bf16),
            pltpu.VMEM((S, D), bf16),
            pltpu.VMEM((D, 3 * D), bf16),
            pltpu.VMEM((D, D), bf16),
            pltpu.VMEM((D, DFF), bf16),
            pltpu.VMEM((DFF, D), bf16),
            pltpu.VMEM((S, D), bf16),
            pltpu.VMEM((2 * D, D), bf16),
            pltpu.VMEM((NG, S, _LANES), bf16),
            pltpu.VMEM((NQ, D, TQ), f32),
            pltpu.VMEM((H, 24, S), f32),
            pltpu.VMEM((NQ, H // 2, 2 * DH, TQ), f32),
            pltpu.VMEM((1, S, TQ), f32),
            pltpu.VMEM((1, S, TQ), f32),
            pltpu.SMEM((1,), jnp.int32),
            pltpu.SemaphoreType.DMA((S // TK,)),
            pltpu.SemaphoreType.DMA((7,)),
            pltpu.SemaphoreType.DMA((S // TR,)),
        ],
        compiler_params=pltpu.CompilerParams(vmem_limit_bytes=100 * 1024 * 1024),
    )(A_x.reshape(S, D), A_wqkv, A_wo, B_w1, B_w2, gate_w)
    return out.reshape(B, S, D)
  return pallas_gated_mix__softmax_full_mha__dense_activation_relu__prompt_kernel

pallas_gated_mix__softmax_full_mha__dense_activation_relu__prompt_kernel = make(U=8)
```

```python
import functools

import jax
import jax.numpy as jnp
from jax import lax
import jax.experimental.pallas as pl
import jax.experimental.pallas.tpu as pltpu

_H = 32
_LOG2E = 1.4426950408889634
_LANES = 128


def _kernel(x_hbm, wqkv_hbm, wo_hbm, w1_hbm, w2_hbm, gw_hbm, out_hbm,
            gw_ref, x_ref, wqkv_ref, wo_ref, w1_ref, w2_ref, out_ref,
            wqvt_ref, k_ref, qm_ref, qf_ref, kf_ref, ks_ref, vt_ref, or_ref, ot_ref,
            kb0, kb1, qb0, qb1, s0, s1, one_ref, z_ref,
            xsem, wsem, osem,
            *, S, D, TQ, TK, TR, TOS, LAG, SC, FORCE_FB, THR, P3GATE, VKS, OGATE, GOFF, QBG, KBG, FINE, KBP):
    H = _H
    DH = D // H
    HPG = _LANES // DH
    NG = -(-H // HPG)
    CK = 128
    def vk_of(c):
        return VKS[c % len(VKS)]

    def kv_base(c):
        return sum(vk_of(cc) for cc in range(c)) // 8
    NQ = S // TQ
    NC = S // CK
    C = TQ // _LANES
    NU = NQ * H
    U = 2 * NQ
    NR = S // TR
    NK = S // TK
    NKV = kv_base(NC)
    f32 = jnp.float32
    bf16 = jnp.bfloat16
    qscale = (DH ** -0.5) * _LOG2E
    nn = (((1,), (0,)), ((), ()))
    nt = (((1,), (1,)), ((), ()))

    def win_start(g):
        return min(g * HPG * DH, D - _LANES)

    def one_lane(g):
        return _LANES - 1 if g < NG - 1 else 0

    def kload(g, k0, k1):
        return pltpu.bitcast(k_ref[g, k0 // 2:k1 // 2, :], bf16)

    def qmload(qi, h):
        return pltpu.bitcast(qm_ref[qi, h], bf16)

    def rows_of(r, t):
        if isinstance(r, int):
            return pl.ds(r * t, t)
        return pl.ds(pl.multiple_of(r * t, t), t)

    def x_copy(r):
        return pltpu.make_async_copy(x_hbm.at[rows_of(r, TK)], x_ref.at[rows_of(r, TK)], xsem.at[r])

    def wqkv_copy(i):
        cols = pl.ds(i * D, D)
        return pltpu.make_async_copy(wqkv_hbm.at[:, cols], wqkv_ref.at[:, cols], wsem.at[i])

    wo_copy = pltpu.make_async_copy(wo_hbm, wo_ref, wsem.at[3])
    w1_copy = pltpu.make_async_copy(w1_hbm, w1_ref, wsem.at[4])
    w2_copy = pltpu.make_async_copy(w2_hbm, w2_ref, wsem.at[5])
    gw_copy = pltpu.make_async_copy(gw_hbm, gw_ref, wsem.at[6])

    NOS = len(TOS)
    OFFS = [sum(TOS[:o]) for o in range(NOS)]
    assert sum(TOS) == TR

    def out_rows(r, o):
        if isinstance(r, int):
            return pl.ds(r * TR + OFFS[o], TOS[o])
        return pl.ds(pl.multiple_of(r * TR + OFFS[o], 64), TOS[o])

    def out_copy(r, o):
        return pltpu.make_async_copy(out_ref.at[out_rows(r, o)], out_hbm.at[out_rows(r, o)], osem.at[r * NOS + o])

    x_copy(0).start()
    wqkv_copy(1).start()
    x_copy(1).start()

    z_ref[0] = 0
    one_ref[...] = jnp.ones_like(one_ref)
    tail_rows = lax.broadcasted_iota(jnp.int32, (H, 8, S), 1)
    vt_ref[:, 16:24, :] = jnp.where(tail_rows == DH - 16, 1.0, 0.0).astype(f32)
    row_id = lax.broadcasted_iota(jnp.int32, (_LANES, TQ), 0)
    lane_k = lax.broadcasted_iota(jnp.int32, (TK, _LANES), 1)
    lane_8 = lax.broadcasted_iota(jnp.int32, (8, _LANES), 1)
    row_8 = lax.broadcasted_iota(jnp.int32, (8, TQ), 0)
    GPK = TK // CK

    def kproj(r):
        rows = rows_of(r, TK)
        kk = jnp.dot(x_ref[rows, :], wqkv_ref[:, D:2 * D], preferred_element_type=f32)
        kk = kk.astype(bf16).astype(f32)
        for g in range(NG):
            w0 = win_start(g)
            kw = jnp.where(lane_k == one_lane(g), 1.0, kk[:, w0:w0 + _LANES])
            k_ref[g, rows_of(r, TK // 2), :] = pltpu.bitcast(kw.astype(bf16), jnp.int32)
        assert GPK % len(VKS) == 0
        VPS = kv_base(GPK)
        for gi in range(GPK):
            VK = vk_of(gi)
            if VK == 0:
                continue
            kv = kk[(gi + 1) * CK - VK:(gi + 1) * CK, :]
            v0 = r * VPS + kv_base(gi)
            dst = pl.ds(v0 * 8, VK) if isinstance(r, int) else pl.ds(pl.multiple_of(v0 * 8, 8), VK)
            for h in range(H):
                kf_ref[h, dst, 0:DH] = kv[:, h * DH:(h + 1) * DH]
            for rr in range(VK // 8):
                for d in range(DH):
                    kb0[v0 + rr, d] = jnp.broadcast_to(kv[rr * 8:(rr + 1) * 8, d:d + 1], (8, _LANES))

    row_16 = lax.broadcasted_iota(jnp.int32, (16, TQ), 0)

    def pack16(v):
        return pltpu.bitcast(v.astype(bf16), jnp.int32)

    def qvproj(r, mid):
        rows = rows_of(r, TQ)
        xr = x_ref[rows, :]
        zq = z_ref[0]
        qt = lax.dot_general(wqvt_ref[0:D, :], xr, nt, preferred_element_type=f32) * qscale
        qt = qt.astype(bf16).astype(f32)
        late = []
        for g in range(NG):
            w0 = win_start(g)
            qw = qt[w0:w0 + _LANES, :]
            zero16 = pack16(jnp.where(row_16 < zq, qw[0:16, :], 0.0))
            for h in range(g * HPG, min((g + 1) * HPG, H)):
                off = h * DH - w0
                qf_ref[r, h, 0:16, :] = qt[h * DH:h * DH + 16, :]
                for tt in range(_LANES // 16):
                    lo, hi = off - 16 * tt, off + DH - 16 * tt
                    val = None
                    if hi > 0 and lo < 16:
                        val = qw[16 * tt:16 * (tt + 1), :]
                        if lo > 0 or hi < 16:
                            val = jnp.where((row_16 >= lo) & (row_16 < hi), val, 0.0)
                    if one_lane(g) // 16 == tt:
                        late.append((g, h, tt, val))
                    elif val is None:
                        qm_ref[r, h, 8 * tt:8 * (tt + 1), :] = zero16
                    else:
                        qm_ref[r, h, 8 * tt:8 * (tt + 1), :] = pack16(val)
        mid()
        s8 = {}
        for g in range(NG):
            w0 = win_start(g)
            h0, h1 = g * HPG, min((g + 1) * HPG, H)
            s8[g] = lax.dot_general(ks_ref[h0 * 8:h1 * 8, :], qt[w0:w0 + _LANES, :].astype(bf16), nn,
                                    preferred_element_type=f32)
        for g, h, tt, val in late:
            hh = h - g * HPG
            m = jnp.max(s8[g][hh * 8:(hh + 1) * 8, :], axis=0, keepdims=True)
            negm = (-m).astype(bf16).astype(f32)
            val = jnp.where(row_16 == one_lane(g) % 16, negm, 0.0 if val is None else val)
            qm_ref[r, h, 8 * tt:8 * (tt + 1), :] = pack16(val)
            t0 = min(h * DH + 16, D - 8)
            tail = qt[t0:t0 + 8, :]
            if t0 != h * DH + 16:
                tail = pltpu.roll(tail, 8 - (h * DH + 16 - t0), 0)
            qf_ref[r, h, 16:24, :] = jnp.where(row_8 == DH - 16, negm, tail)
        HS = H // 2
        for p in range(2):
            r0 = D + p * HS * DH
            vt = lax.dot_general(wqvt_ref[r0:r0 + HS * DH, :], xr, nt, preferred_element_type=f32)
            vt = vt.astype(bf16).astype(f32)
            for hh in range(HS):
                vt_ref[p * HS + hh, 0:DH, rows] = vt[hh * DH:(hh + 1) * DH, :]

    wqkv_copy(1).wait()

    NK1 = NK - NQ

    def k_body(r, c):
        @pl.when(r == 0)
        def _():
            x_copy(2).start()
            wqkv_copy(0).start()
        @pl.when(r == 1)
        def _():
            x_copy(3).start()
            wqkv_copy(2).start()
        @pl.when(r == 2)
        def _():
            x_copy(4).start()
            x_copy(5).start()
        x_copy(r).wait()
        kproj(r)
        return c
    lax.fori_loop(0, NK1 - 1, k_body, 0)
    x_copy(6).start()
    x_copy(7).start()
    x_copy(NK1 - 1).wait()
    wqkv_copy(0).wait()
    wqkv_copy(2).wait()
    wqvt_ref[0:D, :] = wqkv_ref[:, 0:D].T
    wqvt_ref[D:2 * D, :] = wqkv_ref[:, 2 * D:3 * D].T
    for h in range(H):
        g = h // HPG
        off = h * DH - win_start(g)
        k8 = kload(g, 0, 16).astype(f32)[0:8, :]
        ks_ref[h * 8:(h + 1) * 8, :] = jnp.where((lane_8 >= off) & (lane_8 < off + DH), k8, 0.0)
    kproj(NK1 - 1)

    def qv_body(r, c):
        x_copy(NK1 + r).wait()
        qvproj(r, lambda: kproj(NK1 + r))
        return c
    lax.fori_loop(0, NQ, qv_body, 0)

    kbs = (kb0, kb1)
    last_o = [None]
    qbs = (qb0, qb1)

    def gated(val, gate, tmask):
        return val if gate is None else jnp.where(tmask, val, gate)

    def vscores(kb_ref, qb_ref, c, gate_fn, tmask):
        RT = vk_of(c) // 8
        if RT == 0:
            return None
        outs = []
        nb = RT // 2
        for b in range(nb):
            acc = [[qb_ref[DH, :, cc * _LANES:(cc + 1) * _LANES] for cc in range(C)] for _ in range(2)]
            for d in range(DH):
                qb = [qb_ref[d, :, cc * _LANES:(cc + 1) * _LANES] for cc in range(C)]
                for rr in range(2):
                    if gate_fn is None:
                        gate = None
                    elif FINE:
                        gate = gate_fn((b * DH + d) * 2 + rr, nb * DH * 2)
                    else:
                        gate = gate_fn(b * DH + d, nb * DH)
                    kb = gated(kb_ref[kv_base(c) + 2 * b + rr, d], gate, tmask)
                    for cc in range(C):
                        acc[rr][cc] = acc[rr][cc] + kb * qb[cc]
            outs += [jnp.concatenate(acc[rr], axis=1) for rr in range(2)]
        return jnp.concatenate(outs, axis=0)

    def make_qb(qb_ref, h, qi, t, gate, tmask):
        rg, cc = t // C, t % C
        tile = gated(qf_ref[qi, h, rg * 8:(rg + 1) * 8, cc * _LANES:(cc + 1) * _LANES], gate, tmask)
        for rr in range(8):
            d = rg * 8 + rr
            if d <= DH:
                qb_ref[d, :, cc * _LANES:(cc + 1) * _LANES] = jnp.broadcast_to(tile[rr:rr + 1, :], (8, _LANES))

    def make_kb(kb_ref, h, v, gate, tmask, d0=0, d1=DH):
        kf = gated(kf_ref[h, v * 8:(v + 1) * 8, :], gate, tmask)
        for d in range(d0, d1):
            kb_ref[v, d] = jnp.broadcast_to(kf[:, d:d + 1], (8, _LANES))

    def pv(vt, c, p, acc):
        o = lax.dot_general(vt[:, c * CK:(c + 1) * CK], p, nn, preferred_element_type=f32)
        last_o[0] = o
        return o if acc is None else acc + o

    def fin(acc, h, qi, odd):
        l = acc[DH:DH + 1, :]
        o = acc[0:DH, :] * (1.0 / l)
        r0 = DH if odd else 0
        ot_ref[qi, lax.div(h, 2), r0:r0 + DH, :] = o

    NT = 3 * C
    for t in range(NT):
        make_qb(qb0, 0, 0, t, None, None)
    sv_first = vscores(kb0, qb0, 0, None, None)

    def body(j, carry):
        sv, lmax, nanacc = carry
        @pl.when(j == 1)
        def _():
            w1_copy.start()
            w2_copy.start()
            wo_copy.start()
            gw_copy.start()
        tmask = one_ref[...] > 0.0
        heads = [2 * j, 2 * j + 1, jnp.minimum(2 * j + 2, H - 1)]
        steps = [(i, c) for i in range(U) for c in range(NC)]
        pend = []
        accs = {}
        st = {"lmax": lmax, "nan": nanacc}

        def flush(n):
            while len(pend) > n:
                i, c, p = pend.pop(0)
                h = heads[i // NQ]
                accs[i] = pv(vt_ref.at[h], c, p, accs.get(i))
                if c == NC - 1:
                    acc = accs.pop(i)
                    or_ref[i % NQ, h] = acc
                    st["lmax"] = jnp.maximum(st["lmax"], acc[16:24, :])
                    st["nan"] = st["nan"] + (acc[0:8, :] + acc[8:16, :] + acc[16:24, :]) * 0.0

        for t, (i, c) in enumerate(steps):
            hp, qi = i // NQ, i % NQ
            h = heads[hp]
            if c == 0:
                qm = qmload(qi, h)
                g = lax.div(h, HPG)
            MK = CK - vk_of(c)
            s = jnp.dot(kload(g, c * CK, c * CK + MK), qm, preferred_element_type=f32)
            p = jnp.exp2(s if sv is None else jnp.concatenate([s, sv], axis=0)).astype(bf16)
            pend.append((i, c, p))
            last_o[0] = None
            flush(LAG)
            srcs = [(s, rg, cc) for rg in range(MK // 8) for cc in range(C)]
            if last_o[0] is not None and OGATE:
                srcs += [(last_o[0], rg, cc) for rg in range(3) for cc in range(C)]
            srcs = srcs[GOFF:]

            def gate_at(k, n):
                a, rg, cc = srcs[k * len(srcs) // n]
                return a[rg * 8:(rg + 1) * 8, cc * _LANES:(cc + 1) * _LANES]

            i2, c2 = (i, c + 1) if c + 1 < NC else (i + 1, 0)
            inext = i + 1
            if c < NT:
                make_qb(qbs[inext % 2], heads[inext // NQ], inext % NQ, c, gate_at(*QBG), tmask)
            kstep = qi * NC + c
            if KBP:
                per = NKV * DH // (NQ * NC * KBP)
                for q in range(KBP):
                    e0 = (kstep * KBP + q) * per
                    v, d0 = e0 // DH, e0 % DH
                    make_kb(kbs[(hp + 1) % 2], heads[hp + 1], v, gate_at(2 * q + 1, 2 * KBP), tmask, d0, d0 + per)
            else:
              for v in range(kstep * NKV // (NQ * NC), (kstep + 1) * NKV // (NQ * NC)):
                make_kb(kbs[(hp + 1) % 2], heads[hp + 1], v, gate_at(*KBG), tmask)
            sv = vscores(kbs[(i2 // NQ) % 2], qbs[i2 % 2], c2, gate_at, tmask)
        flush(0)
        return sv, st["lmax"], st["nan"]

    _, lmax, nanacc = lax.fori_loop(0, H // 2, body, (sv_first, jnp.zeros((8, TQ), f32), jnp.zeros((8, TQ), f32)))

    okv = (jnp.abs(nanacc) <= 1.0) & ((row_8 != DH - 16) | (lmax <= THR))
    nbad = jnp.max(jnp.where(okv, 0.0, 1.0))
    if FORCE_FB:
        nbad = nbad + 1.0

    @pl.when(nbad > 0.0)
    def _():
        def fb_body(u, carry):
            h = lax.div(u, NQ)
            qi = lax.rem(u, NQ)
            g = lax.div(h, HPG)
            z = z_ref[0]
            qm = qmload(qi, h)
            m = None
            for c in range(NC):
                s = jnp.dot(kload(g, c * CK, (c + 1) * CK), qm, preferred_element_type=f32)
                s0[0, c * CK:(c + 1) * CK, :] = s
                mc = jnp.max(s.reshape(CK // 8, 8, TQ), axis=0)
                m = mc if m is None else jnp.maximum(m, mc)
            m = jnp.max(m, axis=0, keepdims=True)
            acc = None
            for c in range(NC):
                p = jnp.exp2(s0[z, c * CK:(c + 1) * CK, :] - m).astype(bf16)
                acc = pv(vt_ref.at[h], c, p, acc)
            or_ref[qi, h] = acc
            return carry
        lax.fori_loop(0, NU, fb_body, 0)

    w1_copy.wait()
    w2_copy.wait()
    wo_copy.wait()
    gw_copy.wait()
    gw = gw_ref[...].astype(f32).reshape(1, D)

    def p3_body(r, carry):
        rows = rows_of(r, TR)
        xr = x_ref[rows, :]
        hf = jnp.dot(xr, w1_ref[...], preferred_element_type=f32)
        hid = jnp.maximum(hf, 0.0).astype(bf16)
        tmask = one_ref[0:1, :] > 0.0
        gl = jnp.sum(xr.astype(f32) * gw, axis=-1, keepdims=True)
        gate = jax.nn.sigmoid(gl)
        for h in range(H):
            acc = or_ref[r, h]
            l = acc[DH:DH + 1, :]
            if P3GATE:
                ct = h * (hf.shape[1] // _LANES) // H
                gt = hf[(h % 4) * 128:(h % 4) * 128 + 1, ct * _LANES:(ct + 1) * _LANES]
                l = jnp.concatenate([jnp.where(tmask, l[:, cc * _LANES:(cc + 1) * _LANES], gt) for cc in range(C)], axis=1)
            ot_ref[h * DH:(h + 1) * DH, :] = acc[0:DH, :] * (1.0 / l)
        ot_all = ot_ref[...].astype(bf16)
        for o in range(NOS):
            sub = slice(OFFS[o], OFFS[o] + TOS[o])
            b = jnp.dot(hid[sub, :], w2_ref[...], preferred_element_type=f32)
            a = lax.dot_general(ot_all[:, sub], wo_ref[...], (((0,), (0,)), ((), ())),
                                preferred_element_type=f32)
            gs = gate[sub, :]
            out_ref[out_rows(r, o), :] = (gs * a + (1.0 - gs) * b).astype(out_ref.dtype)
            out_copy(r, o).start()
        return carry
    lax.fori_loop(0, NR, p3_body, 0)
    for r in range(NR):
        for o in range(NOS):
            out_copy(r, o).wait()


def make(TQ=512, TK=256, TR=512, TOS=(256, 192, 64), LAG=2, SC=False, FORCE_FB=False, THR=2.0 ** 40, P3GATE=True, VKS=(16,), OGATE=True, GOFF=0, QBG=(0, 1), KBG=(1, 2), FINE=False, KBP=0):
  @jax.jit
  def pallas_gated_mix__softmax_full_mha__dense_activation_relu__prompt_kernel(
    A_x: jax.Array,
    A_wqkv: jax.Array,
    A_wo: jax.Array,
    B_x: jax.Array,
    B_w1: jax.Array,
    B_w2: jax.Array,
    gate_w: jax.Array,
  ):
    del B_x
    B, S, D = A_x.shape
    assert B == 1
    H = _H
    DH = D // H
    DFF = B_w1.shape[1]
    NQ = S // TQ
    NG = -(-H // (_LANES // DH))
    NKV = sum(VKS) * (S // 128 // len(VKS)) // 8
    f32, bf16 = jnp.float32, jnp.bfloat16
    anyspec = pl.BlockSpec(memory_space=pl.ANY)

    out = pl.pallas_call(
        functools.partial(_kernel, S=S, D=D, TQ=TQ, TK=TK, TR=TR, TOS=TOS, LAG=LAG, SC=SC,
                          FORCE_FB=FORCE_FB, THR=THR, P3GATE=P3GATE, VKS=VKS, OGATE=OGATE, GOFF=GOFF, QBG=QBG, KBG=KBG, FINE=FINE, KBP=KBP),
        out_shape=jax.ShapeDtypeStruct((S, D), A_x.dtype),
        in_specs=[anyspec] * 6,
        out_specs=anyspec,
        scratch_shapes=[
            pltpu.VMEM((D,), bf16),
            pltpu.VMEM((S, D), bf16),
            pltpu.VMEM((D, 3 * D), bf16),
            pltpu.VMEM((D, D), bf16),
            pltpu.VMEM((D, DFF), bf16),
            pltpu.VMEM((DFF, D), bf16),
            pltpu.VMEM((S, D), bf16),
            pltpu.VMEM((2 * D, D), bf16),
            pltpu.VMEM((NG, S // 2, _LANES), jnp.int32),
            pltpu.VMEM((NQ, H, _LANES // 2, TQ), jnp.int32),
            pltpu.VMEM((NQ, H, 24, TQ), f32),
            pltpu.VMEM((H, NKV * 8, _LANES), f32),
            pltpu.VMEM((H * 8, _LANES), f32),
            pltpu.VMEM((H, 24, S), f32),
            pltpu.VMEM((NQ, H, 24, TQ), f32),
            pltpu.VMEM((D, TQ), f32),
            pltpu.VMEM((NKV, DH, 8, _LANES), f32),
            pltpu.VMEM((NKV, DH, 8, _LANES), f32),
            pltpu.VMEM((24, 8, TQ), f32),
            pltpu.VMEM((24, 8, TQ), f32),
            pltpu.VMEM((1, S, TQ), f32),
            pltpu.VMEM((24, TQ), f32),
            pltpu.VMEM((8, _LANES), f32),
            pltpu.SMEM((1,), jnp.int32),
            pltpu.SemaphoreType.DMA((S // TK,)),
            pltpu.SemaphoreType.DMA((7,)),
            pltpu.SemaphoreType.DMA((S // TR * len(TOS),)),
        ],
        compiler_params=pltpu.CompilerParams(vmem_limit_bytes=110 * 1024 * 1024),
    )(A_x.reshape(S, D), A_wqkv, A_wo, B_w1, B_w2, gate_w)
    return out.reshape(B, S, D)
  return pallas_gated_mix__softmax_full_mha__dense_activation_relu__prompt_kernel

pallas_gated_mix__softmax_full_mha__dense_activation_relu__prompt_kernel = make(KBP=1)
```

```python
import functools

import jax
import jax.numpy as jnp
from jax import lax
import jax.experimental.pallas as pl
import jax.experimental.pallas.tpu as pltpu

_H = 32
_LOG2E = 1.4426950408889634
_LANES = 128
_TQ = 512
_TK = 256
_TR = 512
_TOS = (256, 192, 64)
_CK = 128
_VK = 16
_LAG = 2
_VP = 8
_L_MAX = 2.0 ** 100
_L_MIN = 2.0 ** -8


def _kernel(x_hbm, wqkv_hbm, wo_hbm, w1_hbm, w2_hbm, gw_hbm, out_hbm,
            gw_ref, x_ref, wqkv_ref, wo_ref, w1_ref, w2_ref, out_ref,
            wqvt_ref, k_ref, qm_ref, qf_ref, kf_ref, ks_ref, vt_ref, or_ref, ot_ref,
            kb0, kb1, qb0, qb1, s0, one_ref, z_ref,
            xsem, wsem, osem, *, S, D):
    H, TQ, TK, TR, TOS, CK, VK, LAG, VP = _H, _TQ, _TK, _TR, _TOS, _CK, _VK, _LAG, _VP
    DH = D // H
    HPG = _LANES // DH
    NG = -(-H // HPG)
    MK = CK - VK
    NQ = S // TQ
    NC = S // CK
    C = TQ // _LANES
    NU = NQ * H
    U = 2 * NQ
    NIT = H // 2
    NR = S // TR
    NK = S // TK
    DFF = w1_ref.shape[1]
    f32 = jnp.float32
    bf16 = jnp.bfloat16
    qscale = (DH ** -0.5) * _LOG2E
    nn = (((1,), (0,)), ((), ()))
    nt = (((1,), (1,)), ((), ()))
    assert NK == 8 and NQ == 4 and TR == TQ and sum(TOS) == TR and VK == 16

    def win_start(g):
        return min(g * HPG * DH, D - _LANES)

    def one_lane(g):
        return _LANES - 1 if g < NG - 1 else 0

    def kload(g, k0, k1):
        return pltpu.bitcast(k_ref[g, k0 // 2:k1 // 2, :], bf16)

    def qmload(qi, h):
        return pltpu.bitcast(qm_ref[qi, h], bf16)

    def pack16(v):
        return pltpu.bitcast(v.astype(bf16), jnp.int32)

    def rows_of(r, t):
        if isinstance(r, int):
            return pl.ds(r * t, t)
        return pl.ds(pl.multiple_of(r * t, t), t)

    def x_copy(r):
        return pltpu.make_async_copy(x_hbm.at[rows_of(r, TK)], x_ref.at[rows_of(r, TK)], xsem.at[r])

    def wqkv_copy(i):
        cols = pl.ds(i * D, D)
        return pltpu.make_async_copy(wqkv_hbm.at[:, cols], wqkv_ref.at[:, cols], wsem.at[i])

    wo_copy = pltpu.make_async_copy(wo_hbm, wo_ref, wsem.at[3])
    w1_copy = pltpu.make_async_copy(w1_hbm, w1_ref, wsem.at[4])
    w2_copy = pltpu.make_async_copy(w2_hbm, w2_ref, wsem.at[5])
    gw_copy = pltpu.make_async_copy(gw_hbm, gw_ref, wsem.at[6])

    NOS = len(TOS)
    OFFS = [sum(TOS[:o]) for o in range(NOS)]

    def out_rows(r, o):
        if isinstance(r, int):
            return pl.ds(r * TR + OFFS[o], TOS[o])
        return pl.ds(pl.multiple_of(r * TR + OFFS[o], 64), TOS[o])

    def out_copy(r, o):
        return pltpu.make_async_copy(out_ref.at[out_rows(r, o)], out_hbm.at[out_rows(r, o)],
                                     osem.at[r * NOS + o])

    x_copy(0).start()
    wqkv_copy(1).start()
    x_copy(1).start()

    z_ref[0] = 0
    one_ref[...] = jnp.ones_like(one_ref)
    tail_rows = lax.broadcasted_iota(jnp.int32, (H, 8, S), 1)
    vt_ref[:, 16:24, :] = jnp.where(tail_rows == DH - 16, 1.0, 0.0).astype(f32)
    lane_k = lax.broadcasted_iota(jnp.int32, (TK, _LANES), 1)
    lane_8 = lax.broadcasted_iota(jnp.int32, (8, _LANES), 1)
    row_8 = lax.broadcasted_iota(jnp.int32, (8, TQ), 0)
    row_16 = lax.broadcasted_iota(jnp.int32, (16, TQ), 0)
    GPK = TK // CK

    def kproj(r):
        rows = rows_of(r, TK)
        kk = jnp.dot(x_ref[rows, :], wqkv_ref[:, D:2 * D], preferred_element_type=f32)
        kk = kk.astype(bf16).astype(f32)
        for g in range(NG):
            w0 = win_start(g)
            kw = jnp.where(lane_k == one_lane(g), 1.0, kk[:, w0:w0 + _LANES])
            k_ref[g, rows_of(r, TK // 2), :] = pack16(kw)
        for gi in range(GPK):
            kv = kk[gi * CK + MK:(gi + 1) * CK, :]
            for h in range(H):
                kf_ref[h, r * GPK + gi] = kv[:, h * DH:(h + 1) * DH]
            for rr in range(2):
                for d in range(DH):
                    kb0[r * GPK + gi, d, rr] = jnp.broadcast_to(
                        kv[rr * 8:(rr + 1) * 8, d:d + 1], (8, _LANES))

    def qvproj(r, mid):
        rows = rows_of(r, TQ)
        xr = x_ref[rows, :]
        zq = z_ref[0]
        qt = lax.dot_general(wqvt_ref[0:D, :], xr, nt, preferred_element_type=f32) * qscale
        qt = qt.astype(bf16).astype(f32)
        late = []
        for g in range(NG):
            w0 = win_start(g)
            qw = qt[w0:w0 + _LANES, :]
            zero16 = pack16(jnp.where(row_16 < zq, qw[0:16, :], 0.0))
            for h in range(g * HPG, min((g + 1) * HPG, H)):
                off = h * DH - w0
                qf_ref[r, h, 0:DH, :] = qt[h * DH:(h + 1) * DH, :]
                for tt in range(_LANES // 16):
                    lo, hi = off - 16 * tt, off + DH - 16 * tt
                    val = None
                    if hi > 0 and lo < 16:
                        val = qw[16 * tt:16 * (tt + 1), :]
                        if lo > 0 or hi < 16:
                            val = jnp.where((row_16 >= lo) & (row_16 < hi), val, 0.0)
                    if one_lane(g) // 16 == tt:
                        late.append((g, h, tt, val))
                    elif val is None:
                        qm_ref[r, h, 8 * tt:8 * (tt + 1), :] = zero16
                    else:
                        qm_ref[r, h, 8 * tt:8 * (tt + 1), :] = pack16(val)
        mid()
        s8 = {}
        for g in range(NG):
            w0 = win_start(g)
            h0, h1 = g * HPG, min((g + 1) * HPG, H)
            s8[g] = lax.dot_general(ks_ref[h0 * 8:h1 * 8, :], qt[w0:w0 + _LANES, :].astype(bf16), nn,
                                    preferred_element_type=f32)
        tm8 = jnp.concatenate([one_ref[...] > 0.0] * C, axis=1)

        def do_late(items, gate):
            for g, h, tt, val in items:
                hh = h - g * HPG
                sh = s8[g][hh * 8:(hh + 1) * 8, :]
                if gate is not None:
                    sh = jnp.where(tm8, sh, gate)
                m = jnp.max(sh, axis=0, keepdims=True)
                negm = (-m).astype(bf16).astype(f32)
                val = jnp.where(row_16 == one_lane(g) % 16, negm, 0.0 if val is None else val)
                qm_ref[r, h, 8 * tt:8 * (tt + 1), :] = pack16(val)
                qf_ref[r, h, DH:24, :] = jnp.broadcast_to(negm, (24 - DH, TQ))

        HS = H // VP
        gate = None
        for p in range(VP):
            do_late(late[p * HS:(p + 1) * HS], gate)
            r0 = D + p * HS * DH
            vt = lax.dot_general(wqvt_ref[r0:r0 + HS * DH, :], xr, nt, preferred_element_type=f32)
            gate = vt[0:8, :]
            vt = vt.astype(bf16).astype(f32)
            for hh in range(HS):
                vt_ref[p * HS + hh, 0:DH, rows] = vt[hh * DH:(hh + 1) * DH, :]

    wqkv_copy(1).wait()

    NK1 = NK - NQ

    def k_body(r, c):
        @pl.when(r == 0)
        def _():
            x_copy(2).start()
            wqkv_copy(0).start()

        @pl.when(r == 1)
        def _():
            x_copy(3).start()
            wqkv_copy(2).start()

        @pl.when(r == 2)
        def _():
            x_copy(4).start()
            x_copy(5).start()
        x_copy(r).wait()
        kproj(r)
        return c
    lax.fori_loop(0, NK1 - 1, k_body, 0)
    x_copy(6).start()
    x_copy(7).start()
    x_copy(NK1 - 1).wait()
    wqkv_copy(0).wait()
    wqkv_copy(2).wait()
    wqvt_ref[0:D, :] = wqkv_ref[:, 0:D].T
    wqvt_ref[D:2 * D, :] = wqkv_ref[:, 2 * D:3 * D].T
    for h in range(H):
        g = h // HPG
        off = h * DH - win_start(g)
        k8 = kload(g, 0, 16).astype(f32)[0:8, :]
        ks_ref[h * 8:(h + 1) * 8, :] = jnp.where((lane_8 >= off) & (lane_8 < off + DH), k8, 0.0)
    kproj(NK1 - 1)

    def qv_body(r, c):
        @pl.when(r == 1)
        def _():
            w1_copy.start()
            w2_copy.start()
            wo_copy.start()
            gw_copy.start()
        x_copy(NK1 + r).wait()
        qvproj(r, lambda: kproj(NK1 + r))
        return c
    lax.fori_loop(0, NQ, qv_body, 0)
    w1_copy.wait()
    w2_copy.wait()
    wo_copy.wait()
    gw_copy.wait()

    kbs = (kb0, kb1)
    qbs = (qb0, qb1)
    NT = 3 * C

    def make_qb(qb_ref, h, qi, t, gate, tmask):
        rg, cc = t // C, t % C
        tile = qf_ref[qi, h, rg * 8:(rg + 1) * 8, cc * _LANES:(cc + 1) * _LANES]
        if gate is not None:
            tile = jnp.where(tmask, tile, gate)
        for rr in range(8):
            d = rg * 8 + rr
            if d <= DH:
                qb_ref[d, cc] = jnp.broadcast_to(tile[rr:rr + 1, :], (8, _LANES))

    def make_kb(kb_ref, h, c, rr, d0, d1, gate, tmask):
        kf = jnp.where(tmask[:, 0:DH], kf_ref[h, c, rr * 8:(rr + 1) * 8, :], gate[:, 0:DH])
        for d in range(d0, d1):
            kb_ref[c, d, rr] = jnp.broadcast_to(kf[:, d:d + 1], (8, _LANES))

    def vscores(i, c, gate_fn, tmask):
        kb_ref, qb_ref = kbs[(i // NQ) % 2], qbs[i % 2]
        acc = jnp.broadcast_to(qb_ref[DH][None], (2, C, 8, _LANES))
        for d in range(DH):
            kb = kb_ref[c, d]
            if gate_fn is not None:
                kb = jnp.where(tmask[None], kb, gate_fn(d, DH)[None])
            acc = acc + kb[:, None] * qb_ref[d][None]
        return acc

    def as_rows(acc):
        return jnp.concatenate(
            [jnp.concatenate([acc[rr, cc] for cc in range(C)], axis=1) for rr in range(2)], axis=0)

    def pv(h, c, p):
        return lax.dot_general(vt_ref[h, :, c * CK:(c + 1) * CK], p, nn, preferred_element_type=f32)

    def tiles(a):
        return [(a, rg, cc) for rg in range(a.shape[0] // 8) for cc in range(a.shape[1] // _LANES)]

    steps = [(i, c) for i in range(U) for c in range(NC)]
    kb_items = [(c, rr, d0, d0 + DH // 2) for c in range(NC) for rr in range(2) for d0 in (0, DH // 2)]
    assert len(kb_items) == NQ * NC

    for t in range(NT):
        make_qb(qb0, 0, 0, t, None, None)
    sv_first = vscores(0, 0, None, None)

    def body(j, carry):
        sv, lmax, lmin, nanacc = carry
        tmask = one_ref[...] > 0.0
        heads = [2 * j, 2 * j + 1, jnp.minimum(2 * j + 2, H - 1)]
        pend = []
        accs = {}
        st = {"lmax": lmax, "lmin": lmin, "nan": nanacc}

        def do_pv():
            i, c, p = pend.pop(0)
            h = heads[i // NQ]
            o = pv(h, c, p)
            accs[i] = o if c == 0 else accs[i] + o
            if c == NC - 1:
                acc = accs.pop(i)
                or_ref[i % NQ, h] = acc
                st["lmax"] = jnp.maximum(st["lmax"], acc[16:24, :])
                st["lmin"] = jnp.minimum(st["lmin"], acc[16:24, :])
                st["nan"] = st["nan"] + (acc[0:8, :] + acc[8:16, :] + acc[16:24, :]) * 0.0
            return o

        for i, c in steps:
            hp, qi = i // NQ, i % NQ
            if c == 0:
                qm = qmload(qi, heads[hp])
                g = lax.div(heads[hp], HPG)
            s = jnp.dot(kload(g, c * CK, c * CK + MK), qm, preferred_element_type=f32)
            p = jnp.exp2(jnp.concatenate([s, as_rows(sv)], axis=0)).astype(bf16)
            pend.append((i, c, p))
            srcs = tiles(s)
            if len(pend) > LAG:
                srcs += tiles(do_pv())

            def gate_at(k, n):
                a, rg, cc = srcs[k * len(srcs) // n]
                return a[rg * 8:(rg + 1) * 8, cc * _LANES:(cc + 1) * _LANES]

            if c < NT:
                make_qb(qbs[(i + 1) % 2], heads[(i + 1) // NQ], (i + 1) % NQ, c, gate_at(0, 1), tmask)
            make_kb(kbs[(hp + 1) % 2], heads[hp + 1], *kb_items[qi * NC + c], gate_at(1, 2), tmask)
            i2, c2 = (i, c + 1) if c + 1 < NC else (i + 1, 0)
            sv = vscores(i2, c2, gate_at, tmask)
        while pend:
            do_pv()
        return sv, st["lmax"], st["lmin"], st["nan"]

    _, lmax, lmin, nanacc = lax.fori_loop(
        0, NIT, body,
        (sv_first, jnp.ones((8, TQ), f32), jnp.ones((8, TQ), f32), jnp.zeros((8, TQ), f32)))

    okv = (jnp.abs(nanacc) <= 1.0) & ((row_8 != DH - 16) | ((lmax <= _L_MAX) & (lmin >= _L_MIN)))
    nbad = jnp.max(jnp.where(okv, 0.0, 1.0))

    @pl.when(nbad > 0.0)
    def _():
        def fb_body(u, carry):
            h = lax.div(u, NQ)
            qi = lax.rem(u, NQ)
            g = lax.div(h, HPG)
            z = z_ref[0]
            qm = qmload(qi, h)
            m = None
            for c in range(NC):
                s = jnp.dot(kload(g, c * CK, (c + 1) * CK), qm, preferred_element_type=f32)
                s0[0, c * CK:(c + 1) * CK, :] = s
                mc = jnp.max(s.reshape(CK // 8, 8, TQ), axis=0)
                m = mc if m is None else jnp.maximum(m, mc)
            m = jnp.max(m, axis=0, keepdims=True)
            acc = None
            for c in range(NC):
                p = jnp.exp2(s0[z, c * CK:(c + 1) * CK, :] - m).astype(bf16)
                o = pv(h, c, p)
                acc = o if acc is None else acc + o
            or_ref[qi, h] = acc
            return carry
        lax.fori_loop(0, NU, fb_body, 0)

    gw = gw_ref[...].astype(f32).reshape(1, D)

    def p3_body(r, carry):
        rows = rows_of(r, TR)
        xr = x_ref[rows, :]
        hf = jnp.dot(xr, w1_ref[...], preferred_element_type=f32)
        hid = jnp.maximum(hf, 0.0).astype(bf16)
        tmask = one_ref[0:1, :] > 0.0
        for h in range(H):
            acc = or_ref[r, h]
            ct = h * (DFF // _LANES) // H
            gt = hf[(h % 4) * 128:(h % 4) * 128 + 1, ct * _LANES:(ct + 1) * _LANES]
            l = jnp.concatenate(
                [jnp.where(tmask, acc[DH:DH + 1, cc * _LANES:(cc + 1) * _LANES], gt) for cc in range(C)],
                axis=1)
            ot_ref[h * DH:(h + 1) * DH, :] = acc[0:DH, :] * (1.0 / l)
        gl = jnp.sum(xr.astype(f32) * gw, axis=-1, keepdims=True)
        gate = jax.nn.sigmoid(gl)
        ot_all = ot_ref[...].astype(bf16)
        for o in range(NOS):
            sub = slice(OFFS[o], OFFS[o] + TOS[o])
            b = jnp.dot(hid[sub, :], w2_ref[...], preferred_element_type=f32)
            a = lax.dot_general(ot_all[:, sub], wo_ref[...], (((0,), (0,)), ((), ())),
                                preferred_element_type=f32)
            gs = gate[sub, :]
            out_ref[out_rows(r, o), :] = (gs * a + (1.0 - gs) * b).astype(out_ref.dtype)
            out_copy(r, o).start()
        return carry
    lax.fori_loop(0, NR, p3_body, 0)
    for r in range(NR):
        for o in range(NOS):
            out_copy(r, o).wait()


@jax.jit
def pallas_gated_mix__softmax_full_mha__dense_activation_relu__prompt_kernel(
    A_x: jax.Array,
    A_wqkv: jax.Array,
    A_wo: jax.Array,
    B_x: jax.Array,
    B_w1: jax.Array,
    B_w2: jax.Array,
    gate_w: jax.Array,
):
    del B_x
    B, S, D = A_x.shape
    assert B == 1
    H, TQ = _H, _TQ
    DH = D // H
    DFF = B_w1.shape[1]
    NQ = S // TQ
    NG = -(-H // (_LANES // DH))
    NC = S // _CK
    f32, bf16, i32 = jnp.float32, jnp.bfloat16, jnp.int32
    anyspec = pl.BlockSpec(memory_space=pl.ANY)

    out = pl.pallas_call(
        functools.partial(_kernel, S=S, D=D),
        out_shape=jax.ShapeDtypeStruct((S, D), A_x.dtype),
        in_specs=[anyspec] * 6,
        out_specs=anyspec,
        scratch_shapes=[
            pltpu.VMEM((D,), bf16),
            pltpu.VMEM((S, D), bf16),
            pltpu.VMEM((D, 3 * D), bf16),
            pltpu.VMEM((D, D), bf16),
            pltpu.VMEM((D, DFF), bf16),
            pltpu.VMEM((DFF, D), bf16),
            pltpu.VMEM((S, D), bf16),
            pltpu.VMEM((2 * D, D), bf16),
            pltpu.VMEM((NG, S // 2, _LANES), i32),
            pltpu.VMEM((NQ, H, _LANES // 2, TQ), i32),
            pltpu.VMEM((NQ, H, 24, TQ), f32),
            pltpu.VMEM((H, NC, _VK, DH), f32),
            pltpu.VMEM((H * 8, _LANES), f32),
            pltpu.VMEM((H, 24, S), f32),
            pltpu.VMEM((NQ, H, 24, TQ), f32),
            pltpu.VMEM((D, TQ), f32),
            pltpu.VMEM((NC, DH, 2, 8, _LANES), f32),
            pltpu.VMEM((NC, DH, 2, 8, _LANES), f32),
            pltpu.VMEM((24, TQ // _LANES, 8, _LANES), f32),
            pltpu.VMEM((24, TQ // _LANES, 8, _LANES), f32),
            pltpu.VMEM((1, S, TQ), f32),
            pltpu.VMEM((8, _LANES), f32),
            pltpu.SMEM((1,), i32),
            pltpu.SemaphoreType.DMA((S // _TK,)),
            pltpu.SemaphoreType.DMA((7,)),
            pltpu.SemaphoreType.DMA((S // _TR * len(_TOS),)),
        ],
        compiler_params=pltpu.CompilerParams(vmem_limit_bytes=110 * 1024 * 1024),
    )(A_x.reshape(S, D), A_wqkv, A_wo, B_w1, B_w2, gate_w)
    return out.reshape(B, S, D)
```
